```python
import jax
import jax.numpy as jnp

def _softmax(x, axis=-1):
    return jax.nn.softmax(x, axis=axis)
def _gelu(x):
    return jax.nn.gelu(x, approximate=True)
def _silu(x):
    return jax.nn.silu(x)
def _sigmoid(x):
    return jax.nn.sigmoid(x)
def _layernorm(x, axis=-1, eps=1e-5):
    m = jnp.mean(x, axis=axis, keepdims=True)
    v = jnp.var(x, axis=axis, keepdims=True)
    return (x - m) / jnp.sqrt(v + eps)
def _scatter_add(tgt, idx, src, axis=0):
    return tgt.at[idx].add(src)
def _segment_sum(src, seg, n):
    return jax.ops.segment_sum(src, seg, n)
class _Rng:
    def __init__(self, key):
        self._k = key
    def _next(self):
        self._k, sub = jax.random.split(self._k)
        return sub
    def normal(self, shape):
        return jax.random.normal(self._next(), shape, dtype=jnp.bfloat16)
    def randint(self, lo, hi, shape):
        return jax.random.randint(self._next(), shape, lo, hi, dtype=jnp.int32)
    def uniform(self, shape, lo=0.0, hi=1.0):
        return jax.random.uniform(self._next(), shape, jnp.bfloat16, lo, hi)
    def permutation(self, n):
        return jax.random.permutation(self._next(), n)


kernel_name = 'parallel_sum__sliding_block_cached__glu_gated_swiglu__decode'

def setup_inputs():
    _rng = _Rng(jax.random.key(int.from_bytes(__import__("os").urandom(4), "little")))
    _w = (lambda a: (lambda t: t.astype(jnp.bfloat16) if jnp.issubdtype(t.dtype, jnp.floating) else t)(jnp.asarray(a)))
    def _A_setup():
        B, Sq, D = 4, 1, 640
        Hq, Hkv, Sk, Dh = 32, 32, 8192, 192
        assert Hq % Hkv == 0, (Hq, Hkv)
        return {
            "x": _w((lambda *s: _rng.normal(s) * 0.05)(B, Sq, D)),
            "k_cache": _w((lambda *s: _rng.normal(s) * 0.05)(B, Hkv, Sk, Dh)),
            "v_cache": _w((lambda *s: _rng.normal(s) * 0.05)(B, Hkv, Sk, Dh)),
            "wq": _w((lambda *s: _rng.normal(s) * 0.05)(D, Hq * Dh) * (D ** -0.5)),
            "wo": _w((lambda *s: _rng.normal(s) * 0.05)(Hq * Dh, D) * ((Hq * Dh) ** -0.5)),
        }
    _A_in = _A_setup()

    def _B_setup():
        B, S, D, F = 4, 1, 640, 1536
        return {
            "x": _w((lambda *s: _rng.normal(s) * 0.05)(B, S, D)),
            "w1": _w((lambda *s: _rng.normal(s) * 0.05)(D, F) * (2.0 / D) ** 0.5),
            "w3": _w((lambda *s: _rng.normal(s) * 0.05)(D, F) * (2.0 / D) ** 0.5),
            "w2": _w((lambda *s: _rng.normal(s) * 0.05)(F, D) * (2.0 / F) ** 0.5),
        }
    _B_in = _B_setup()

    return {
        "A_x": _A_in["x"],
        "A_k_cache": _A_in["k_cache"],
        "A_v_cache": _A_in["v_cache"],
        "A_wq": _A_in["wq"],
        "A_wo": _A_in["wo"],
        "B_x": _B_in["x"],
        "B_w1": _B_in["w1"],
        "B_w3": _B_in["w3"],
        "B_w2": _B_in["w2"],
    }

def reference(A_x, A_k_cache, A_v_cache, A_wq, A_wo, B_x, B_w1, B_w3, B_w2):
    def _A_ref(x, k_cache, v_cache, wq, wo):
        B, Sq, D = x.shape
        Hq, Dh = 32, 192
        Hkv, Sk = k_cache.shape[1], k_cache.shape[2]
        W = min(4096, max(256, Sk // 4))
        rep = Hq // Hkv
        q = (lambda x, *d: x.transpose(*d))((x @ wq).reshape(B, Sq, Hq, Dh), 0, 2, 1, 3)
        k = jnp.repeat(k_cache[:, :, Sk - W:, :], rep, axis=1)
        v = jnp.repeat(v_cache[:, :, Sk - W:, :], rep, axis=1)
        scores = jnp.einsum("bhqd,bhkd->bhqk", q, k) * (Dh ** -0.5)
        p = _softmax(scores, axis=-1)
        o = jnp.einsum("bhqk,bhkd->bhqd", p, v)
        return (lambda x, *d: x.transpose(*d))(o, 0, 2, 1, 3).reshape(B, Sq, Hq * Dh) @ wo

    def _B_ref(x, w1, w3, w2):
        gate = jnp.einsum("bsd,df->bsf", x, w1)
        up = jnp.einsum("bsd,df->bsf", x, w3)
        h = _silu(gate) * up
        out = jnp.einsum("bsf,fd->bsd", h, w2)
        return out

    x = A_x
    xn = _layernorm(x, axis=-1)
    return x + _A_ref(xn, A_k_cache, A_v_cache, A_wq, A_wo) + _B_ref(xn, B_w1, B_w3, B_w2)
```

```python
import jax
import jax.numpy as jnp
import jax.experimental.pallas as pl
import jax.experimental.pallas.tpu as pltpu

HQ, DH = 32, 192
HG = 8
NBUF = 4
KSPLIT = 2
WPOS = 2


@jax.jit
def pallas_parallel_sum__sliding_block_cached__glu_gated_swiglu__decode_kernel(
    A_x, A_k_cache, A_v_cache, A_wq, A_wo, B_x, B_w1, B_w3, B_w2,
):
    del B_x
    B, Sq, D = A_x.shape
    _, H, Sk, _ = A_k_cache.shape
    W = min(4096, max(256, Sk // 4))
    F = B_w1.shape[1]
    R = HG * DH
    NG = H // HG
    NU = NG * B
    RS = R // KSPLIT
    scale = DH ** -0.5
    bf = jnp.bfloat16
    f32 = jnp.float32

    kt = jnp.swapaxes(A_k_cache, 2, 3).reshape(B * H * DH, Sk)
    vt = jnp.swapaxes(A_v_cache, 2, 3).reshape(B * H * DH, Sk)
    x2 = A_x.reshape(B * Sq, D)

    def kern(x_ref, kt_hbm, vt_hbm, wq_hbm, wo_hbm, w1_hbm, w3_hbm, w2_hbm,
             o_ref, kbuf, vbuf, wq, wo, w1, w3, w2, q_s, o_s, ksem, vsem, wsem):
        def unit(u):
            return u % B, u // B

        def copies(u, hbm, buf, sem):
            b, g = unit(u)
            r0 = (b * H + g * HG) * DH
            slot = u % NBUF
            return [
                pltpu.make_async_copy(
                    hbm.at[pl.ds(r0 + i * RS, RS), pl.ds(Sk - W, W)],
                    buf.at[slot, pl.ds(i * RS, RS)],
                    sem.at[slot, i])
                for i in range(KSPLIT)
            ]

        def start(u):
            for c in copies(u, kt_hbm, kbuf, ksem):
                c.start()
            for c in copies(u, vt_hbm, vbuf, vsem):
                c.start()

        cq = pltpu.make_async_copy(wq_hbm, wq, wsem.at[0])
        c1 = pltpu.make_async_copy(w1_hbm, w1, wsem.at[1])
        c3 = pltpu.make_async_copy(w3_hbm, w3, wsem.at[2])
        c2 = pltpu.make_async_copy(w2_hbm, w2, wsem.at[3])
        co = pltpu.make_async_copy(wo_hbm, wo, wsem.at[4])
        cq.start()
        for u in range(min(NBUF, NU)):
            start(u)

        def late():
            co.start(); c1.start(); c3.start(); c2.start()

        x = x_ref[...].astype(f32)
        m = jnp.mean(x, axis=-1, keepdims=True)
        xc = x - m
        v = jnp.mean(xc * xc, axis=-1, keepdims=True)
        xn = (xc / jnp.sqrt(v + 1e-5)).astype(bf)

        cq.wait()
        q_s[...] = jnp.zeros(q_s.shape, f32)
        q_s[0:B, :] = jnp.dot(xn, wq[...], preferred_element_type=f32)
        o_s[...] = jnp.zeros(o_s.shape, f32)

        row = jax.lax.broadcasted_iota(jnp.int32, (HG, R), 0)
        col = jax.lax.broadcasted_iota(jnp.int32, (HG, R), 1)
        diag = (col >= row * DH) & (col < (row + 1) * DH)

        acc = jnp.zeros((B, D), f32)
        for u in range(NU):
            b, g = unit(u)
            slot = u % NBUF
            q = q_s[b:b + 1, g * R:(g + 1) * R]
            qd = jnp.where(diag, jnp.broadcast_to(q, (HG, R)), 0.0).astype(bf)
            for c in copies(u, kt_hbm, kbuf, ksem):
                c.wait()
            s = jnp.dot(qd, kbuf[slot], preferred_element_type=f32) * scale
            mx = jnp.max(s, axis=-1, keepdims=True)
            e = jnp.exp(s - mx)
            l = jnp.sum(e, axis=-1, keepdims=True)
            p = e.astype(bf)
            vc = copies(u, vt_hbm, vbuf, vsem)
            outs = []
            for i in range(KSPLIT):
                vc[i].wait()
                outs.append(jax.lax.dot_general(
                    p, vbuf[slot, i * RS:(i + 1) * RS, :],
                    (((1,), (1,)), ((), ())), preferred_element_type=f32))
            if u + NBUF < NU:
                start(u + NBUF)
            if u == WPOS:
                late()
            o = jnp.concatenate(outs, axis=1) / l
            o = jnp.sum(jnp.where(diag, o, 0.0), axis=0, keepdims=True)
            o_s[b:b + 1, g * R:(g + 1) * R] = o

            if u == NU - B - 1:
                c1.wait(); c3.wait(); c2.wait()
                gate = jnp.dot(xn, w1[...], preferred_element_type=f32)
                up = jnp.dot(xn, w3[...], preferred_element_type=f32)
                h = (gate * jax.nn.sigmoid(gate) * up).astype(bf)
                acc = acc + jnp.dot(h, w2[...], preferred_element_type=f32)
                co.wait()
                n = (NG - 1) * R
                acc = acc + jnp.dot(o_s[0:B, 0:n].astype(bf), wo[0:n, :],
                                    preferred_element_type=f32)
        n = (NG - 1) * R
        acc = acc + jnp.dot(o_s[0:B, n:].astype(bf), wo[n:, :],
                            preferred_element_type=f32)
        o_ref[...] = (x + acc).astype(o_ref.dtype)

    hbm = pl.BlockSpec(memory_space=pl.ANY)
    out = pl.pallas_call(
        kern,
        out_shape=jax.ShapeDtypeStruct((B * Sq, D), A_x.dtype),
        in_specs=[pl.BlockSpec(memory_space=pltpu.VMEM)] + [hbm] * 7,
        out_specs=pl.BlockSpec(memory_space=pltpu.VMEM),
        scratch_shapes=[
            pltpu.VMEM((NBUF, R, W), bf), pltpu.VMEM((NBUF, R, W), bf),
            pltpu.VMEM(A_wq.shape, bf), pltpu.VMEM(A_wo.shape, bf),
            pltpu.VMEM((D, F), bf), pltpu.VMEM((D, F), bf), pltpu.VMEM((F, D), bf),
            pltpu.VMEM((8, H * DH), f32), pltpu.VMEM((8, H * DH), f32),
            pltpu.SemaphoreType.DMA((NBUF, KSPLIT)),
            pltpu.SemaphoreType.DMA((NBUF, KSPLIT)),
            pltpu.SemaphoreType.DMA((5,)),
        ],
        compiler_params=pltpu.CompilerParams(vmem_limit_bytes=120 * 1024 * 1024),
    )(x2, kt, vt, A_wq, A_wo, B_w1, B_w3, B_w2)
    return out.reshape(B, Sq, D)
```

```python
import jax
import jax.numpy as jnp
import jax.experimental.pallas as pl
import jax.experimental.pallas.tpu as pltpu

HQ, DH = 32, 192
HG = 4
NBUF = 3
KSPLIT = 1
WPOS = 12


@jax.jit
def pallas_parallel_sum__sliding_block_cached__glu_gated_swiglu__decode_kernel(
    A_x, A_k_cache, A_v_cache, A_wq, A_wo, B_x, B_w1, B_w3, B_w2,
):
    del B_x
    B, Sq, D = A_x.shape
    _, H, Sk, _ = A_k_cache.shape
    W = min(4096, max(256, Sk // 4))
    F = B_w1.shape[1]
    R = HG * DH
    NG = H // HG
    NU = NG * B
    RS = R // KSPLIT
    scale = DH ** -0.5
    bf = jnp.bfloat16
    f32 = jnp.float32

    kt = jnp.swapaxes(A_k_cache, 2, 3).reshape(B * H * DH, Sk)
    vt = jnp.swapaxes(A_v_cache, 2, 3).reshape(B * H * DH, Sk)
    x2 = A_x.reshape(B * Sq, D)

    def kern(x_ref, kt_hbm, vt_hbm, wq_hbm, wo_hbm, w1_hbm, w3_hbm, w2_hbm,
             o_ref, kbuf, vbuf, wq, wo, w1, w3, w2, q_s, o_s, ksem, vsem, wsem):
        def unit(u):
            return u % B, u // B

        def copies(u, hbm, buf, sem):
            b, g = unit(u)
            r0 = (b * H + g * HG) * DH
            slot = u % NBUF
            return [
                pltpu.make_async_copy(
                    hbm.at[pl.ds(r0 + i * RS, RS), pl.ds(Sk - W, W)],
                    buf.at[slot, pl.ds(i * RS, RS)],
                    sem.at[slot, i])
                for i in range(KSPLIT)
            ]

        def start(u):
            for c in copies(u, kt_hbm, kbuf, ksem):
                c.start()
            for c in copies(u, vt_hbm, vbuf, vsem):
                c.start()

        cq = pltpu.make_async_copy(wq_hbm, wq, wsem.at[0])
        c1 = pltpu.make_async_copy(w1_hbm, w1, wsem.at[1])
        c3 = pltpu.make_async_copy(w3_hbm, w3, wsem.at[2])
        c2 = pltpu.make_async_copy(w2_hbm, w2, wsem.at[3])
        co = pltpu.make_async_copy(wo_hbm, wo, wsem.at[4])
        cq.start()
        for u in range(min(NBUF, NU)):
            start(u)

        def late():
            co.start(); c1.start(); c3.start(); c2.start()

        x = x_ref[...].astype(f32)
        m = jnp.mean(x, axis=-1, keepdims=True)
        xc = x - m
        v = jnp.mean(xc * xc, axis=-1, keepdims=True)
        xn = (xc / jnp.sqrt(v + 1e-5)).astype(bf)

        cq.wait()
        q_s[...] = jnp.zeros(q_s.shape, f32)
        q_s[0:B, :] = jnp.dot(xn, wq[...], preferred_element_type=f32)
        o_s[...] = jnp.zeros(o_s.shape, f32)

        row = jax.lax.broadcasted_iota(jnp.int32, (HG, R), 0)
        col = jax.lax.broadcasted_iota(jnp.int32, (HG, R), 1)
        diag = (col >= row * DH) & (col < (row + 1) * DH)

        acc = jnp.zeros((B, D), f32)
        for u in range(NU):
            b, g = unit(u)
            slot = u % NBUF
            q = q_s[b:b + 1, g * R:(g + 1) * R]
            qd = jnp.where(diag, jnp.broadcast_to(q, (HG, R)), 0.0).astype(bf)
            for c in copies(u, kt_hbm, kbuf, ksem):
                c.wait()
            s = jnp.dot(qd, kbuf[slot], preferred_element_type=f32) * scale
            mx = jnp.max(s, axis=-1, keepdims=True)
            e = jnp.exp(s - mx)
            l = jnp.sum(e, axis=-1, keepdims=True)
            p = e.astype(bf)
            vc = copies(u, vt_hbm, vbuf, vsem)
            outs = []
            for i in range(KSPLIT):
                vc[i].wait()
                outs.append(jax.lax.dot_general(
                    p, vbuf[slot, i * RS:(i + 1) * RS, :],
                    (((1,), (1,)), ((), ())), preferred_element_type=f32))
            if u + NBUF < NU:
                start(u + NBUF)
            if u == WPOS:
                late()
            o = jnp.concatenate(outs, axis=1) / l
            o = jnp.sum(jnp.where(diag, o, 0.0), axis=0, keepdims=True)
            o_s[b:b + 1, g * R:(g + 1) * R] = o

            if u == NU - B - 1:
                c1.wait(); c3.wait(); c2.wait()
                gate = jnp.dot(xn, w1[...], preferred_element_type=f32)
                up = jnp.dot(xn, w3[...], preferred_element_type=f32)
                h = (gate * jax.nn.sigmoid(gate) * up).astype(bf)
                acc = acc + jnp.dot(h, w2[...], preferred_element_type=f32)
                co.wait()
                n = (NG - 1) * R
                acc = acc + jnp.dot(o_s[0:B, 0:n].astype(bf), wo[0:n, :],
                                    preferred_element_type=f32)
        n = (NG - 1) * R
        acc = acc + jnp.dot(o_s[0:B, n:].astype(bf), wo[n:, :],
                            preferred_element_type=f32)
        o_ref[...] = (x + acc).astype(o_ref.dtype)

    hbm = pl.BlockSpec(memory_space=pl.ANY)
    out = pl.pallas_call(
        kern,
        out_shape=jax.ShapeDtypeStruct((B * Sq, D), A_x.dtype),
        in_specs=[pl.BlockSpec(memory_space=pltpu.VMEM)] + [hbm] * 7,
        out_specs=pl.BlockSpec(memory_space=pltpu.VMEM),
        scratch_shapes=[
            pltpu.VMEM((NBUF, R, W), bf), pltpu.VMEM((NBUF, R, W), bf),
            pltpu.VMEM(A_wq.shape, bf), pltpu.VMEM(A_wo.shape, bf),
            pltpu.VMEM((D, F), bf), pltpu.VMEM((D, F), bf), pltpu.VMEM((F, D), bf),
            pltpu.VMEM((8, H * DH), f32), pltpu.VMEM((8, H * DH), f32),
            pltpu.SemaphoreType.DMA((NBUF, KSPLIT)),
            pltpu.SemaphoreType.DMA((NBUF, KSPLIT)),
            pltpu.SemaphoreType.DMA((5,)),
        ],
        compiler_params=pltpu.CompilerParams(vmem_limit_bytes=120 * 1024 * 1024),
    )(x2, kt, vt, A_wq, A_wo, B_w1, B_w3, B_w2)
    return out.reshape(B, Sq, D)
```

```python
import jax
import jax.numpy as jnp
import jax.experimental.pallas as pl
import jax.experimental.pallas.tpu as pltpu

HQ, DH = 32, 192
HG = 2
NBUF = 3
KSPLIT = 1
WPOS = 8


@jax.jit
def pallas_parallel_sum__sliding_block_cached__glu_gated_swiglu__decode_kernel(
    A_x, A_k_cache, A_v_cache, A_wq, A_wo, B_x, B_w1, B_w3, B_w2,
):
    del B_x
    B, Sq, D = A_x.shape
    _, H, Sk, _ = A_k_cache.shape
    W = min(4096, max(256, Sk // 4))
    F = B_w1.shape[1]
    R = HG * DH
    NG = H // HG
    NU = NG * B
    RS = R // KSPLIT
    scale = DH ** -0.5
    bf = jnp.bfloat16
    f32 = jnp.float32

    kt = jnp.swapaxes(A_k_cache, 2, 3).reshape(B * H * DH, Sk)
    vt = jnp.swapaxes(A_v_cache, 2, 3).reshape(B * H * DH, Sk)
    x2 = A_x.reshape(B * Sq, D)

    def kern(x_hbm, kt_hbm, vt_hbm, wq_hbm, wo_hbm, w1_hbm, w3_hbm, w2_hbm,
             o_ref, x_ref, kbuf, vbuf, wq, wo, w1, w3, w2, q_s, o_s, ksem, vsem, wsem):
        def unit(u):
            return u % B, u // B

        def copies(u, hbm, buf, sem):
            b, g = unit(u)
            r0 = (b * H + g * HG) * DH
            slot = u % NBUF
            return [
                pltpu.make_async_copy(
                    hbm.at[pl.ds(r0 + i * RS, RS), pl.ds(Sk - W, W)],
                    buf.at[slot, pl.ds(i * RS, RS)],
                    sem.at[slot, i])
                for i in range(KSPLIT)
            ]

        def start(u):
            for c in copies(u, kt_hbm, kbuf, ksem):
                c.start()
            for c in copies(u, vt_hbm, vbuf, vsem):
                c.start(priority=1)

        cq = pltpu.make_async_copy(wq_hbm, wq, wsem.at[0])
        c1 = pltpu.make_async_copy(w1_hbm, w1, wsem.at[1])
        c3 = pltpu.make_async_copy(w3_hbm, w3, wsem.at[2])
        c2 = pltpu.make_async_copy(w2_hbm, w2, wsem.at[3])
        co = pltpu.make_async_copy(wo_hbm, wo, wsem.at[4])
        cx = pltpu.make_async_copy(x_hbm, x_ref, wsem.at[5])
        cq.start()
        cx.start()
        for u in range(min(NBUF, NU)):
            start(u)

        def late():
            co.start(); c1.start(); c3.start(); c2.start()

        cx.wait()
        x = x_ref[...].astype(f32)
        m = jnp.mean(x, axis=-1, keepdims=True)
        xc = x - m
        v = jnp.mean(xc * xc, axis=-1, keepdims=True)
        xn = (xc / jnp.sqrt(v + 1e-5)).astype(bf)

        cq.wait()
        q_s[...] = jnp.zeros(q_s.shape, f32)
        q_s[0:B, :] = jnp.dot(xn, wq[...], preferred_element_type=f32)
        o_s[...] = jnp.zeros(o_s.shape, f32)

        row = jax.lax.broadcasted_iota(jnp.int32, (HG, R), 0)
        col = jax.lax.broadcasted_iota(jnp.int32, (HG, R), 1)
        diag = (col >= row * DH) & (col < (row + 1) * DH)

        acc = jnp.zeros((B, D), f32)
        for u in range(NU):
            b, g = unit(u)
            slot = u % NBUF
            q = q_s[b:b + 1, g * R:(g + 1) * R]
            qd = jnp.where(diag, jnp.broadcast_to(q, (HG, R)), 0.0).astype(bf)
            for c in copies(u, kt_hbm, kbuf, ksem):
                c.wait()
            s = jnp.dot(qd, kbuf[slot], preferred_element_type=f32) * scale
            mx = jnp.max(s, axis=-1, keepdims=True)
            e = jnp.exp(s - mx)
            l = jnp.sum(e, axis=-1, keepdims=True)
            p = e.astype(bf)
            vc = copies(u, vt_hbm, vbuf, vsem)
            outs = []
            for i in range(KSPLIT):
                vc[i].wait()
                outs.append(jax.lax.dot_general(
                    p, vbuf[slot, i * RS:(i + 1) * RS, :],
                    (((1,), (1,)), ((), ())), preferred_element_type=f32))
            if u + NBUF < NU:
                start(u + NBUF)
            if u == WPOS:
                late()
            o = jnp.concatenate(outs, axis=1) / l
            o = jnp.sum(jnp.where(diag, o, 0.0), axis=0, keepdims=True)
            o_s[b:b + 1, g * R:(g + 1) * R] = o

            if u == NU - B - 1:
                c1.wait(); c3.wait(); c2.wait()
                gate = jnp.dot(xn, w1[...], preferred_element_type=f32)
                up = jnp.dot(xn, w3[...], preferred_element_type=f32)
                h = (gate * jax.nn.sigmoid(gate) * up).astype(bf)
                acc = acc + jnp.dot(h, w2[...], preferred_element_type=f32)
                co.wait()
                n = (NG - 1) * R
                acc = acc + jnp.dot(o_s[0:B, 0:n].astype(bf), wo[0:n, :],
                                    preferred_element_type=f32)
        n = (NG - 1) * R
        acc = acc + jnp.dot(o_s[0:B, n:].astype(bf), wo[n:, :],
                            preferred_element_type=f32)
        o_ref[...] = (x + acc).astype(o_ref.dtype)

    hbm = pl.BlockSpec(memory_space=pl.ANY)
    out = pl.pallas_call(
        kern,
        out_shape=jax.ShapeDtypeStruct((B * Sq, D), A_x.dtype),
        in_specs=[hbm] * 8,
        out_specs=pl.BlockSpec(memory_space=pltpu.VMEM),
        scratch_shapes=[
            pltpu.VMEM((B * Sq, D), bf),
            pltpu.VMEM((NBUF, R, W), bf), pltpu.VMEM((NBUF, R, W), bf),
            pltpu.VMEM(A_wq.shape, bf), pltpu.VMEM(A_wo.shape, bf),
            pltpu.VMEM((D, F), bf), pltpu.VMEM((D, F), bf), pltpu.VMEM((F, D), bf),
            pltpu.VMEM((8, H * DH), f32), pltpu.VMEM((8, H * DH), f32),
            pltpu.SemaphoreType.DMA((NBUF, KSPLIT)),
            pltpu.SemaphoreType.DMA((NBUF, KSPLIT)),
            pltpu.SemaphoreType.DMA((6,)),
        ],
        compiler_params=pltpu.CompilerParams(vmem_limit_bytes=120 * 1024 * 1024),
    )(x2, kt, vt, A_wq, A_wo, B_w1, B_w3, B_w2)
    return out.reshape(B, Sq, D)
```
